```python
import os as _os
_os.environ.setdefault("JAX_PLATFORMS", "cpu")
import jax
import jax.numpy as jnp

def _softmax(x, axis=-1):
    return jax.nn.softmax(x, axis=axis)
def _gelu(x):
    return jax.nn.gelu(x, approximate=True)
def _silu(x):
    return jax.nn.silu(x)
def _sigmoid(x):
    return jax.nn.sigmoid(x)
def _layernorm(x, axis=-1, eps=1e-5):
    m = jnp.mean(x, axis=axis, keepdims=True)
    v = jnp.var(x, axis=axis, keepdims=True)
    return (x - m) / jnp.sqrt(v + eps)
def _scatter_add(tgt, idx, src, axis=0):
    return tgt.at[idx].add(src)
def _segment_sum(src, seg, n):
    return jax.ops.segment_sum(src, seg, n)
class _Rng:
    def __init__(self, key):
        self._k = key
    def _next(self):
        self._k, sub = jax.random.split(self._k)
        return sub
    def normal(self, shape):
        return jax.random.normal(self._next(), shape, dtype=jnp.bfloat16)
    def randint(self, lo, hi, shape):
        return jax.random.randint(self._next(), shape, lo, hi, dtype=jnp.int32)
    def uniform(self, shape, lo=0.0, hi=1.0):
        return jax.random.uniform(self._next(), shape, jnp.bfloat16, lo, hi)
    def permutation(self, n):
        return jax.random.permutation(self._next(), n)


kernel_name = 'sequential_preLN__mha_block__moe_arch_mod__prompt'

def setup_inputs():
    _rng = _Rng(jax.random.key(int.from_bytes(__import__("os").urandom(4), "little")))
    _w = (lambda a: (lambda t: t.astype(jnp.bfloat16) if jnp.issubdtype(t.dtype, jnp.floating) else t)(jnp.asarray(a)))
    def _A_setup():
        B, S, D, H = 1, 2048, 640, 32
        return {
            "x": _w((lambda *s: _rng.normal(s) * 0.05)(B, S, D)),
            "wqkv": _w((lambda *s: _rng.normal(s) * 0.05)(D, 3 * D)),
            "wo": _w((lambda *s: _rng.normal(s) * 0.05)(D, D)),
        }
    _A_in = _A_setup()

    def _B_setup():
        B, S, D, F, C = 1, 2048, 640, 1536, 1
        return {
            "x": _w((lambda *s: _rng.normal(s) * 0.05)(B, S, D)),
            "w_r": _w((lambda *s: _rng.normal(s) * 0.05)(D)),
            "w_gate": _w((lambda *s: _rng.normal(s) * 0.05)(D, F)),
            "w_up": _w((lambda *s: _rng.normal(s) * 0.05)(D, F)),
            "w_down": _w((lambda *s: _rng.normal(s) * 0.05)(F, D)),
        }
    _B_in = _B_setup()

    return {
        "A_x": _A_in["x"],
        "A_wqkv": _A_in["wqkv"],
        "A_wo": _A_in["wo"],
        "B_x": _B_in["x"],
        "B_w_r": _B_in["w_r"],
        "B_w_gate": _B_in["w_gate"],
        "B_w_up": _B_in["w_up"],
        "B_w_down": _B_in["w_down"],
    }

def reference(A_x, A_wqkv, A_wo, B_x, B_w_r, B_w_gate, B_w_up, B_w_down):
    def _A_ref(x, wqkv, wo):
        B, S, D = x.shape
        H = 32
        Dh = D // H
        qkv = (lambda x, *d: x.transpose(*d))((x @ wqkv).reshape(B, S, 3, H, Dh), 2, 0, 3, 1, 4)
        q, k, v = qkv[0], qkv[1], qkv[2]
        scores = jnp.einsum("bhqd,bhkd->bhqk", q, k) * (Dh ** -0.5)
        p = _softmax(scores, axis=-1)
        o = jnp.einsum("bhqk,bhkd->bhqd", p, v)
        return (lambda x, *d: x.transpose(*d))(o, 0, 2, 1, 3).reshape(B, S, D) @ wo

    def _B_ref(x, w_r, w_gate, w_up, w_down):
        B, S, D = x.shape
        C = 1
        r = x @ w_r
        idx = jnp.argsort(-r, axis=-1)[:, :C]
        idx_e = jnp.repeat(idx.reshape(B, C, 1), D, axis=2)
        x_sel = jnp.take_along_axis(x, idx_e, axis=1)
        g = _silu(x_sel @ w_gate)
        u = x_sel @ w_up
        y = (g * u) @ w_down
        r_sel = _sigmoid(jnp.take_along_axis(r, idx, axis=1))
        y = y * r_sel.reshape(B, C, 1)
        b_off = (jnp.arange(B) * S).reshape(B, 1)
        flat_idx = (idx + b_off).reshape(B * C)
        zero = (x * 0.0).reshape(B * S, D)
        upd = _scatter_add(zero, flat_idx, y.reshape(B * C, D), axis=0)
        return x + upd.reshape(B, S, D)

    x = A_x
    h = x + _A_ref(_layernorm(x, axis=-1), A_wqkv, A_wo)
    h2 = h + _B_ref(_layernorm(h, axis=-1), B_w_r, B_w_gate, B_w_up, B_w_down)
    return h2
```

```python
import functools
import math

import jax
import jax.numpy as jnp
import jax.experimental.pallas as pl
import jax.experimental.pallas.tpu as pltpu

S, D, H, DH, F = 2048, 640, 32, 20, 1536
HP = 32
DP = H * HP
TQ = 512
CK = 128
NC = S // CK
CH = 512
EPS = 1e-5
QSCALE = (DH ** -0.5) * math.log2(math.e)
F32 = jnp.float32
BF16 = jnp.bfloat16


def _head_window(h):
    lo = DH * h
    if lo % 128 + DH <= 128:
        return False, lo // 128, lo % 128
    return True, (lo - 64) // 128, (lo - 64) % 128


def _ln(x):
    m = jnp.mean(x, axis=-1, keepdims=True)
    xc = x - m
    v = jnp.mean(xc * xc, axis=-1, keepdims=True)
    return xc * jax.lax.rsqrt(v + EPS)


def _kernel(x_ref, wqkv_ref, wo_ref, wr_ref, wg_hbm, wu_hbm, wd_hbm, o_ref,
            q_sc, k_sc, sta_sc, stb_sc, m_sc, at_sc, v_sc,  ln2_sc, wg_ref, wu_ref, wd_ref,
            sems, bestv_sc, besti_sc):
    i = pl.program_id(0)
    nsteps = pl.num_programs(0)

    def ffn_copies():
        return (pltpu.make_async_copy(wg_hbm, wg_ref, sems.at[0]),
                pltpu.make_async_copy(wu_hbm, wu_ref, sems.at[1]),
                pltpu.make_async_copy(wd_hbm, wd_ref, sems.at[2]))

    @pl.when(i == 0)
    def _():
        for cp in ffn_copies():
            cp.start()
        wvt = wqkv_ref[:, 2 * D:].astype(F32).T.astype(BF16)
        wqt = wqkv_ref[:, :D].astype(F32).T.astype(BF16)
        sub = jax.lax.broadcasted_iota(jnp.int32, (HP - DH, CH), 0)
        ones_pad = jnp.where(sub == 0, 1.0, 0.0).astype(F32)

        def body(c, carry):
            rows = pl.ds(pl.multiple_of(c * CH, CH), CH)
            xn32 = _ln(x_ref[rows, :].astype(F32))
            xn = xn32.astype(BF16)
            xnt = xn32.T.astype(BF16)
            qt = jnp.dot(wqt, xnt, preferred_element_type=F32)
            q_sc[:, rows] = (qt * QSCALE).astype(BF16)
            k = jnp.dot(xn, wqkv_ref[:, D:2 * D], preferred_element_type=F32)
            kb = k.astype(BF16)
            for w in range(5):
                k_sc[w, rows, :] = kb[:, w * 128:(w + 1) * 128]
            ksb = k[:, 64:576].astype(BF16)
            for w in range(4):
                k_sc[5 + w, rows, :] = ksb[:, w * 128:(w + 1) * 128]
            vt = jnp.dot(wvt, xnt, preferred_element_type=F32)
            vt_rows = []
            for h in range(H):
                vt_rows += [vt[DH * h:DH * (h + 1)], ones_pad]
            v_sc[:, rows] = jnp.concatenate(vt_rows, axis=0).astype(BF16)
            return carry
        jax.lax.fori_loop(0, S // CH, body, 0)
        bestv_sc[0] = -jnp.inf
        besti_sc[0] = 0

    qrows = pl.ds(pl.multiple_of(i * TQ, TQ), TQ)
    sub128 = jax.lax.broadcasted_iota(jnp.int32, (128, TQ), 0)

    def qk(h, c, qb):
        qcols = pl.ds(pl.multiple_of(qb * TQ, TQ), TQ)
        lo = h * DH
        shifted = (lo % 128) > (128 - DH)
        lo2 = jnp.where(shifted, lo - 64, lo)
        w = lo2 // 128
        off = lo2 % 128
        r0 = pl.multiple_of(w * 128 + jnp.where(shifted, 64, 0), 64)
        qg = q_sc[pl.ds(r0, 128), qcols]
        qm = jnp.where((sub128 >= off) & (sub128 < off + DH), qg, jnp.zeros_like(qg))
        widx = w + jnp.where(shifted, 5, 0)
        kc = k_sc[widx, c * CK:(c + 1) * CK, :]
        st = jnp.dot(kc, qm, preferred_element_type=F32)
        mc = jnp.max(st.reshape(CK // 8, 8, TQ), axis=0)
        return st, mc

    def head(h, cur_ref, m, nxt_ref, hn, qbn):
        mnext = None
        ot = None
        vrow = h * HP if isinstance(h, int) else pl.multiple_of(h * HP, HP)
        for c in range(NC):
            st_n, mc = qk(hn, c, qbn)
            nxt_ref[c * CK:(c + 1) * CK, :] = st_n
            mnext = mc if mnext is None else jnp.maximum(mnext, mc)
            pt = jnp.exp2(cur_ref[c * CK:(c + 1) * CK, :] - m).astype(BF16)
            vh = v_sc[pl.ds(vrow, HP), c * CK:(c + 1) * CK]
            d = jnp.dot(vh, pt, preferred_element_type=F32)
            ot = d if ot is None else ot + d
        l = ot[DH:DH + 1, :]
        return ot[:DH] * (1.0 / l), jnp.max(mnext, axis=0, keepdims=True)

    @pl.when(i == 0)
    def _():
        m0 = None
        for c in range(NC):
            st_n, mc = qk(0, c, 0)
            sta_sc[c * CK:(c + 1) * CK, :] = st_n
            m0 = mc if m0 is None else jnp.maximum(m0, mc)
        m_sc[...] = jnp.max(m0, axis=0, keepdims=True)

    def pair(t, m, qb_last):
        oa, m1 = head(2 * t, sta_sc, m, stb_sc, 2 * t + 1, i)
        if qb_last is None:
            ob, m2 = head(2 * t + 1, stb_sc, m1, sta_sc, 2 * t + 2, i)
            arow = pl.multiple_of(t * (2 * DH), 8)
        else:
            ob, m2 = head(2 * t + 1, stb_sc, m1, sta_sc, 0, qb_last)
            arow = t * (2 * DH)
        at_sc[pl.ds(arow, 2 * DH), :] = jnp.concatenate([oa, ob], axis=0)
        return m2

    m = jax.lax.fori_loop(0, H // 2 - 1, lambda t, m: pair(t, m, None), m_sc[...])
    m_sc[...] = pair(H // 2 - 1, m, jnp.minimum(i + 1, nsteps - 1))
    attn_t = at_sc[...]
    attn = attn_t.T.astype(BF16)
    a = jnp.dot(attn, wo_ref[...], preferred_element_type=F32)
    h = (x_ref[qrows, :].astype(F32) + a).astype(BF16).astype(F32)
    ln2 = _ln(h).astype(BF16).astype(F32)
    ln2_sc[qrows, :] = ln2
    o_ref[qrows, :] = (h + ln2).astype(BF16)
    r = jnp.sum(ln2 * wr_ref[...].astype(F32), axis=-1, keepdims=True)
    r = r.astype(BF16).astype(F32)
    bmax = jnp.max(r)
    ridx = jax.lax.broadcasted_iota(jnp.int32, (TQ, 1), 0) + i * TQ
    bidx = jnp.min(jnp.where(r == bmax, ridx, S))

    @pl.when(bmax > bestv_sc[0])
    def _():
        bestv_sc[0] = bmax
        besti_sc[0] = bidx

    @pl.when(i == nsteps - 1)
    def _():
        for cp in ffn_copies():
            cp.wait()
        idx = besti_sc[0]
        rsel = bestv_sc[0]
        xs = jnp.broadcast_to(ln2_sc[pl.ds(idx, 1), :], (8, D)).astype(BF16)
        gt = jnp.dot(xs, wg_ref[...], preferred_element_type=F32)
        up = jnp.dot(xs, wu_ref[...], preferred_element_type=F32)
        act = (gt * jax.nn.sigmoid(gt) * up).astype(BF16)
        y = jnp.dot(act, wd_ref[...], preferred_element_type=F32)
        y = y * jax.nn.sigmoid(jnp.full((1, 1), rsel, F32))
        base = pl.multiple_of((idx // 16) * 16, 16)
        rows = pl.ds(base, 16)
        sub = jax.lax.broadcasted_iota(jnp.int32, (16, D), 0) + base
        y16 = jnp.concatenate([y, y], axis=0)
        cur = o_ref[rows, :].astype(F32)
        o_ref[rows, :] = jnp.where(sub == idx, cur + y16, cur).astype(BF16)


@jax.jit
def pallas_sequential_preLN__mha_block__moe_arch_mod__prompt_kernel(
    A_x, A_wqkv, A_wo, B_x, B_w_r, B_w_gate, B_w_up, B_w_down,
):
    x = A_x.reshape(S, D)
    wr = B_w_r.reshape(1, D)
    full = lambda shape: pl.BlockSpec(shape, lambda i: (0,) * len(shape))
    anyspec = pl.BlockSpec(memory_space=pl.ANY)
    out = pl.pallas_call(
        _kernel,
        grid=(S // TQ,),
        in_specs=[full((S, D)), full((D, 3 * D)), full((D, D)), full((1, D)),
                  anyspec, anyspec, anyspec],
        out_specs=full((S, D)),
        out_shape=jax.ShapeDtypeStruct((S, D), BF16),
        scratch_shapes=[
            pltpu.VMEM((D, S), BF16),
            pltpu.VMEM((9, S, 128), BF16),
            pltpu.VMEM((S, TQ), F32),
            pltpu.VMEM((S, TQ), F32),
            pltpu.VMEM((1, TQ), F32),
            pltpu.VMEM((D, TQ), F32),
            pltpu.VMEM((DP, S), BF16),
            pltpu.VMEM((S, D), F32),
            pltpu.VMEM((D, F), BF16),
            pltpu.VMEM((D, F), BF16),
            pltpu.VMEM((F, D), BF16),
            pltpu.SemaphoreType.DMA((3,)),
            pltpu.SMEM((1,), F32),
            pltpu.SMEM((1,), jnp.int32),
        ],
        compiler_params=pltpu.CompilerParams(
            dimension_semantics=("arbitrary",),
            vmem_limit_bytes=100 * 1024 * 1024,
        ),
    )(x, A_wqkv, A_wo, wr, B_w_gate, B_w_up, B_w_down)
    return out.reshape(1, S, D)
```

```python
import math

import jax
import jax.numpy as jnp
import jax.experimental.pallas as pl
import jax.experimental.pallas.tpu as pltpu

S, D, H, DH, F = 2048, 640, 32, 20, 1536
HP = 32
DP = H * HP
TQ = 512
CK = 128
NC = S // CK
CH = 512
EPS = 1e-5
QSCALE = (DH ** -0.5) * math.log2(math.e)
F32 = jnp.float32
BF16 = jnp.bfloat16


def _ln(x):
    m = jnp.mean(x, axis=-1, keepdims=True)
    xc = x - m
    v = jnp.mean(xc * xc, axis=-1, keepdims=True)
    return xc * jax.lax.rsqrt(v + EPS)


def _kernel(x_hbm, wqkv_hbm, wo_hbm, wr_ref, wg_hbm, wu_hbm, wd_hbm, o_hbm,
            x_ref, wqkv_ref, wo_ref, o_ref,
            q_sc, k_sc, sta_sc, stb_sc, m_sc, at_sc, v_sc,  ln2_sc, wg_ref, wu_ref, wd_ref,
            sems, xsems, osems, bestv_sc, besti_sc):
    i = pl.program_id(0)
    nsteps = pl.num_programs(0)

    def ffn_copies():
        return (pltpu.make_async_copy(wg_hbm, wg_ref, sems.at[0]),
                pltpu.make_async_copy(wu_hbm, wu_ref, sems.at[1]),
                pltpu.make_async_copy(wd_hbm, wd_ref, sems.at[2]))

    def x_copy(c):
        rows = pl.ds(pl.multiple_of(c * CH, CH), CH)
        return pltpu.make_async_copy(x_hbm.at[rows, :], x_ref.at[rows, :], xsems.at[c])

    def out_copy(b):
        rows = pl.ds(pl.multiple_of(b * TQ, TQ), TQ)
        return pltpu.make_async_copy(o_ref.at[rows, :], o_hbm.at[rows, :], osems.at[b])

    wqkv_copy = pltpu.make_async_copy(wqkv_hbm, wqkv_ref, sems.at[3])
    wo_copy = pltpu.make_async_copy(wo_hbm, wo_ref, sems.at[4])

    @pl.when(i == 0)
    def _():
        wqkv_copy.start()
        for c in range(S // CH):
            x_copy(c).start()
        wo_copy.start()
        for cp in ffn_copies():
            cp.start()
        wqkv_copy.wait()
        wvt = wqkv_ref[:, 2 * D:].astype(F32).T.astype(BF16)
        wqt = wqkv_ref[:, :D].astype(F32).T.astype(BF16)
        sub = jax.lax.broadcasted_iota(jnp.int32, (HP - DH, CH), 0)
        ones_pad = jnp.where(sub == 0, 1.0, 0.0).astype(F32)

        def body(c, carry):
            rows = pl.ds(pl.multiple_of(c * CH, CH), CH)
            x_copy(c).wait()
            xn32 = _ln(x_ref[rows, :].astype(F32))
            xn = xn32.astype(BF16)
            xnt = xn32.T.astype(BF16)
            qt = jnp.dot(wqt, xnt, preferred_element_type=F32)
            q_sc[:, rows] = (qt * QSCALE).astype(BF16)
            k = jnp.dot(xn, wqkv_ref[:, D:2 * D], preferred_element_type=F32)
            kb = k.astype(BF16)
            for w in range(5):
                k_sc[w, rows, :] = kb[:, w * 128:(w + 1) * 128]
            ksb = k[:, 64:576].astype(BF16)
            for w in range(4):
                k_sc[5 + w, rows, :] = ksb[:, w * 128:(w + 1) * 128]
            vt = jnp.dot(wvt, xnt, preferred_element_type=F32)
            vt_rows = []
            for h in range(H):
                vt_rows += [vt[DH * h:DH * (h + 1)], ones_pad]
            v_sc[:, rows] = jnp.concatenate(vt_rows, axis=0).astype(BF16)
            return carry
        jax.lax.fori_loop(0, S // CH, body, 0)
        wo_copy.wait()
        bestv_sc[0] = -jnp.inf
        besti_sc[0] = 0

    qrows = pl.ds(pl.multiple_of(i * TQ, TQ), TQ)
    sub128 = jax.lax.broadcasted_iota(jnp.int32, (128, TQ), 0)

    def qk(h, c, qb):
        qcols = pl.ds(pl.multiple_of(qb * TQ, TQ), TQ)
        lo = h * DH
        shifted = (lo % 128) > (128 - DH)
        lo2 = jnp.where(shifted, lo - 64, lo)
        w = lo2 // 128
        off = lo2 % 128
        r0 = pl.multiple_of(w * 128 + jnp.where(shifted, 64, 0), 64)
        qg = q_sc[pl.ds(r0, 128), qcols]
        qm = jnp.where((sub128 >= off) & (sub128 < off + DH), qg, jnp.zeros_like(qg))
        widx = w + jnp.where(shifted, 5, 0)
        kc = k_sc[widx, c * CK:(c + 1) * CK, :]
        st = jnp.dot(kc, qm, preferred_element_type=F32)
        mc = jnp.max(st.reshape(CK // 8, 8, TQ), axis=0)
        return st, mc

    def head(h, cur_ref, m, nxt_ref, hn, qbn):
        mnext = None
        ot = None
        vrow = h * HP if isinstance(h, int) else pl.multiple_of(h * HP, HP)
        for c in range(NC):
            st_n, mc = qk(hn, c, qbn)
            nxt_ref[c * CK:(c + 1) * CK, :] = st_n
            mnext = mc if mnext is None else jnp.maximum(mnext, mc)
            pt = jnp.exp2(cur_ref[c * CK:(c + 1) * CK, :] - m).astype(BF16)
            vh = v_sc[pl.ds(vrow, HP), c * CK:(c + 1) * CK]
            d = jnp.dot(vh, pt, preferred_element_type=F32)
            ot = d if ot is None else ot + d
        l = ot[DH:DH + 1, :]
        return ot[:DH] * (1.0 / l), jnp.max(mnext, axis=0, keepdims=True)

    @pl.when(i == 0)
    def _():
        m0 = None
        for c in range(NC):
            st_n, mc = qk(0, c, 0)
            sta_sc[c * CK:(c + 1) * CK, :] = st_n
            m0 = mc if m0 is None else jnp.maximum(m0, mc)
        m_sc[...] = jnp.max(m0, axis=0, keepdims=True)

    def pair(t, m, qb_last):
        oa, m1 = head(2 * t, sta_sc, m, stb_sc, 2 * t + 1, i)
        if qb_last is None:
            ob, m2 = head(2 * t + 1, stb_sc, m1, sta_sc, 2 * t + 2, i)
            arow = pl.multiple_of(t * (2 * DH), 8)
        else:
            ob, m2 = head(2 * t + 1, stb_sc, m1, sta_sc, 0, qb_last)
            arow = t * (2 * DH)
        at_sc[pl.ds(arow, 2 * DH), :] = jnp.concatenate([oa, ob], axis=0)
        return m2

    m = jax.lax.fori_loop(0, H // 2 - 1, lambda t, m: pair(t, m, None), m_sc[...], unroll=5)
    m_sc[...] = pair(H // 2 - 1, m, jnp.minimum(i + 1, nsteps - 1))
    attn_t = at_sc[...]
    attn = attn_t.T.astype(BF16)
    a = jnp.dot(attn, wo_ref[...], preferred_element_type=F32)
    h = (x_ref[qrows, :].astype(F32) + a).astype(BF16).astype(F32)
    ln2 = _ln(h).astype(BF16).astype(F32)
    ln2_sc[qrows, :] = ln2
    o_ref[qrows, :] = (h + ln2).astype(BF16)
    r = jnp.sum(ln2 * wr_ref[...].astype(F32), axis=-1, keepdims=True)
    r = r.astype(BF16).astype(F32)
    bmax = jnp.max(r)
    ridx = jax.lax.broadcasted_iota(jnp.int32, (TQ, 1), 0) + i * TQ
    bidx = jnp.min(jnp.where(r == bmax, ridx, S))

    @pl.when(bmax > bestv_sc[0])
    def _():
        bestv_sc[0] = bmax
        besti_sc[0] = bidx

    @pl.when(i < nsteps - 1)
    def _():
        out_copy(i).start()

    @pl.when(i == nsteps - 1)
    def _():
        for cp in ffn_copies():
            cp.wait()
        for b in range(S // TQ - 1):
            out_copy(b).wait()
        idx = besti_sc[0]
        rsel = bestv_sc[0]
        xs = jnp.broadcast_to(ln2_sc[pl.ds(idx, 1), :], (8, D)).astype(BF16)
        gt = jnp.dot(xs, wg_ref[...], preferred_element_type=F32)
        up = jnp.dot(xs, wu_ref[...], preferred_element_type=F32)
        act = (gt * jax.nn.sigmoid(gt) * up).astype(BF16)
        y = jnp.dot(act, wd_ref[...], preferred_element_type=F32)
        y = y * jax.nn.sigmoid(jnp.full((1, 1), rsel, F32))
        base = pl.multiple_of((idx // 16) * 16, 16)
        rows = pl.ds(base, 16)
        sub = jax.lax.broadcasted_iota(jnp.int32, (16, D), 0) + base
        y16 = jnp.concatenate([y, y], axis=0)
        cur = o_ref[rows, :].astype(F32)
        o_ref[rows, :] = jnp.where(sub == idx, cur + y16, cur).astype(BF16)
        last = out_copy(S // TQ - 1)
        last.start()
        last.wait()
        fix = pltpu.make_async_copy(o_ref.at[rows, :], o_hbm.at[rows, :], osems.at[0])
        fix.start()
        fix.wait()


@jax.jit
def pallas_sequential_preLN__mha_block__moe_arch_mod__prompt_kernel(
    A_x, A_wqkv, A_wo, B_x, B_w_r, B_w_gate, B_w_up, B_w_down,
):
    x = A_x.reshape(S, D)
    wr = B_w_r.reshape(1, D)
    full = lambda shape: pl.BlockSpec(shape, lambda i: (0,) * len(shape))
    anyspec = pl.BlockSpec(memory_space=pl.ANY)
    out = pl.pallas_call(
        _kernel,
        grid=(S // TQ,),
        in_specs=[anyspec, anyspec, anyspec, full((1, D)),
                  anyspec, anyspec, anyspec],
        out_specs=anyspec,
        out_shape=jax.ShapeDtypeStruct((S, D), BF16),
        scratch_shapes=[
            pltpu.VMEM((S, D), BF16),
            pltpu.VMEM((D, 3 * D), BF16),
            pltpu.VMEM((D, D), BF16),
            pltpu.VMEM((S, D), BF16),
            pltpu.VMEM((D, S), BF16),
            pltpu.VMEM((9, S, 128), BF16),
            pltpu.VMEM((S, TQ), F32),
            pltpu.VMEM((S, TQ), F32),
            pltpu.VMEM((1, TQ), F32),
            pltpu.VMEM((D, TQ), F32),
            pltpu.VMEM((DP, S), BF16),
            pltpu.VMEM((S, D), F32),
            pltpu.VMEM((D, F), BF16),
            pltpu.VMEM((D, F), BF16),
            pltpu.VMEM((F, D), BF16),
            pltpu.SemaphoreType.DMA((5,)),
            pltpu.SemaphoreType.DMA((S // CH,)),
            pltpu.SemaphoreType.DMA((S // TQ,)),
            pltpu.SMEM((1,), F32),
            pltpu.SMEM((1,), jnp.int32),
        ],
        compiler_params=pltpu.CompilerParams(
            dimension_semantics=("arbitrary",),
            vmem_limit_bytes=100 * 1024 * 1024,
        ),
    )(x, A_wqkv, A_wo, wr, B_w_gate, B_w_up, B_w_down)
    return out.reshape(1, S, D)
```
